```python
import os as _os
_os.environ.setdefault("JAX_PLATFORMS", "cpu")
import jax
import jax.numpy as jnp

def _softmax(x, axis=-1):
    return jax.nn.softmax(x, axis=axis)
def _gelu(x):
    return jax.nn.gelu(x, approximate=True)
def _silu(x):
    return jax.nn.silu(x)
def _sigmoid(x):
    return jax.nn.sigmoid(x)
def _layernorm(x, axis=-1, eps=1e-5):
    m = jnp.mean(x, axis=axis, keepdims=True)
    v = jnp.var(x, axis=axis, keepdims=True)
    return (x - m) / jnp.sqrt(v + eps)
def _scatter_add(tgt, idx, src, axis=0):
    return tgt.at[idx].add(src)
def _segment_sum(src, seg, n):
    return jax.ops.segment_sum(src, seg, n)
class _Rng:
    def __init__(self, key):
        self._k = key
    def _next(self):
        self._k, sub = jax.random.split(self._k)
        return sub
    def normal(self, shape):
        return jax.random.normal(self._next(), shape, dtype=jnp.bfloat16)
    def randint(self, lo, hi, shape):
        return jax.random.randint(self._next(), shape, lo, hi, dtype=jnp.int32)
    def uniform(self, shape, lo=0.0, hi=1.0):
        return jax.random.uniform(self._next(), shape, jnp.bfloat16, lo, hi)
    def permutation(self, n):
        return jax.random.permutation(self._next(), n)


kernel_name = 'concat_heads__gqa_block_cached__mha_block_cached__near_ridge'

def setup_inputs():
    _rng = _Rng(jax.random.key(int.from_bytes(__import__("os").urandom(4), "little")))
    _w = (lambda a: (lambda t: t.astype(jnp.bfloat16) if jnp.issubdtype(t.dtype, jnp.floating) else t)(jnp.asarray(a)))
    def _A_setup():
        B, Sq, D = 8, 112, 448
        Hq, Hkv, Sk, Dh = 16, 8, 512, 256
        assert Hq % Hkv == 0, (Hq, Hkv)
        return {
            "x": _w((lambda *s: _rng.normal(s) * 0.8)(B, Sq, D)),
            "k_cache": _w((lambda *s: _rng.normal(s) * 0.8)(B, Hkv, Sk, Dh)),
            "v_cache": _w((lambda *s: _rng.normal(s) * 0.05)(B, Hkv, Sk, Dh)),
            "wq": _w((lambda *s: _rng.normal(s) * 0.8)(D, Hq * Dh) * (D ** -0.5)),
            "wo": _w((lambda *s: _rng.normal(s) * 0.05)(Hq * Dh, D) * ((Hq * Dh) ** -0.5)),
        }
    _A_in = _A_setup()

    def _B_setup():
        B, Sq, D = 8, 112, 448
        H, Sk, Dh = 16, 512, 256
        return {
            "x": _w((lambda *s: _rng.normal(s) * 0.8)(B, Sq, D)),
            "k_cache": _w((lambda *s: _rng.normal(s) * 0.8)(B, H, Sk, Dh)),
            "v_cache": _w((lambda *s: _rng.normal(s) * 0.05)(B, H, Sk, Dh)),
            "wq": _w((lambda *s: _rng.normal(s) * 0.8)(D, H * Dh) * (D ** -0.5)),
            "wo": _w((lambda *s: _rng.normal(s) * 0.05)(H * Dh, D) * ((H * Dh) ** -0.5)),
        }
    _B_in = _B_setup()

    return {
        "A_x": _A_in["x"],
        "A_k_cache": _A_in["k_cache"],
        "A_v_cache": _A_in["v_cache"],
        "A_wq": _A_in["wq"],
        "A_wo": _A_in["wo"],
        "B_x": _B_in["x"],
        "B_k_cache": _B_in["k_cache"],
        "B_v_cache": _B_in["v_cache"],
        "B_wq": _B_in["wq"],
        "B_wo": _B_in["wo"],
    }

def reference(A_x, A_k_cache, A_v_cache, A_wq, A_wo, B_x, B_k_cache, B_v_cache, B_wq, B_wo):
    def _A_ref(x, k_cache, v_cache, wq, wo):
        B, Sq, D = x.shape
        Hq, Dh = 16, 256
        Hkv = k_cache.shape[1]
        rep = Hq // Hkv
        q = (lambda x, *d: x.transpose(*d))((x @ wq).reshape(B, Sq, Hq, Dh), 0, 2, 1, 3)
        k = jnp.repeat(k_cache, rep, axis=1)
        v = jnp.repeat(v_cache, rep, axis=1)
        scores = jnp.einsum("bhqd,bhkd->bhqk", q, k) * (Dh ** -0.5)
        p = _softmax(scores, axis=-1)
        o = jnp.einsum("bhqk,bhkd->bhqd", p, v)
        return (lambda x, *d: x.transpose(*d))(o, 0, 2, 1, 3).reshape(B, Sq, Hq * Dh) @ wo

    def _B_ref(x, k_cache, v_cache, wq, wo):
        B, Sq, D = x.shape
        H, Dh = 16, 256
        q = (lambda x, *d: x.transpose(*d))((x @ wq).reshape(B, Sq, H, Dh), 0, 2, 1, 3)
        scores = jnp.einsum("bhqd,bhkd->bhqk", q, k_cache) * (Dh ** -0.5)
        p = _softmax(scores, axis=-1)
        o = jnp.einsum("bhqk,bhkd->bhqd", p, v_cache)
        return (lambda x, *d: x.transpose(*d))(o, 0, 2, 1, 3).reshape(B, Sq, H * Dh) @ wo

    a = _A_ref(A_x, A_k_cache, A_v_cache, A_wq, A_wo)
    b = _B_ref(B_x, B_k_cache, B_v_cache, B_wq, B_wo)
    return jnp.concatenate([a, b], axis=-1)
```

```python
import jax, jax.numpy as jnp, numpy as np
from jax import lax
from jax.experimental import pallas as pl
from jax.experimental.pallas import tpu as pltpu

NT = (((1,), (1,)), ((), ()))
C = float(np.log2(np.e) / 16.0)
bf, f32 = jnp.bfloat16, jnp.float32

def build(D=3, chunks=(0,2,4,6,8), nodma=False, nowait=False, la=1, od=3, flags=None, late_a=True, rows=(0,128,384,640,896),
          xsplit=True, pad=384, u32=False, qmode=0, resched=True, wpad=0, interpret=False):
    flags = dict(flags or {})
    if resched: flags['XLA_TPU_RESCHEDULE_DMA_DONES'] = True
    R = D + 1
    nc = len(chunks) - 1
    def kernel(xA,kA,vA,wqA,woA,xB,kB,vB,wqB,woB,out, kr, vr, xb, wq, wo, qb, obuf, acc, outb, sk, sv, sq, so, sx, sout):
        srcs = ((xA,kA,vA,wqA,woA,1), (xB,kB,vB,wqB,woB,2))
        def c_x(br, h): return pltpu.make_async_copy(srcs[br][0].at[h*448:(h+1)*448], xb.at[br, h*448:(h+1)*448], sx.at[br, h])
        def c_wq(src, g, s, j):
            return pltpu.make_async_copy(src.at[:, pl.ds(pl.multiple_of(g*512 + j*256, 256), 256)], wq.at[s, :, j*256:(j+1)*256], sq.at[s, j])
        def c_wo(src, g, s):
            return pltpu.make_async_copy(src.at[:, pl.ds(pl.multiple_of(g*512, 512), 512)], wo.at[s, :, 0:512], so.at[s])
        def c_kv(src, dst, sem, nh, g, s, c):
            b0, b1 = chunks[c], chunks[c+1]
            return pltpu.make_async_copy(src.at[b0:b1, pl.ds(g*nh, nh)], dst.at[s, b0:b1, pl.ds(0, nh), :, 0:256], sem.at[s, c])
        def c_out(r0, r1, c0, c1, k):
            return pltpu.make_async_copy(outb.at[r0:r1, c0:c1], out.at[r0:r1, c0:c1], sout.at[k])
        wo_after = min(c for c in range(nc) if chunks[c+1] > min(od, 7) - 1)
        def issue_br(br, g, s, first=False):
            _, k, v, q_, o_, nh = srcs[br]
            c_wq(q_, g, s, 0).start()
            if first: c_x(0, 0).start(); c_x(0, 1).start()
            c_wq(q_, g, s, 1).start()
            for c in range(nc):
                c_kv(k, kr, sk, nh, g, s, c).start()
                c_kv(v, vr, sv, nh, g, s, c).start()
                if c == wo_after: c_wo(o_, g, s).start()
        def issue(i):
            s = i % R
            @pl.when(i < 8)
            def _(): issue_br(0, jnp.minimum(i, 7), s)
            @pl.when(i == 8)
            def _(): c_x(1, 0).start(); c_x(1, 1).start()
            @pl.when(jnp.logical_and(i >= 8, i < 16))
            def _(): issue_br(1, jnp.clip(i - 8, 0, 7), s)

        def scores(q, k): return lax.dot_general(q, k, NT, preferred_element_type=f32)
        def pv(s, v):
            m = jnp.max(s, axis=-1, keepdims=True)
            p = jnp.exp2((s - m) * C)
            l = jnp.sum(p, axis=-1, keepdims=True)
            r = pl.reciprocal(l, approx=True)
            r = r * (2.0 - l * r)
            o = jnp.dot(p.astype(bf), v, preferred_element_type=f32)
            return (o * r).astype(bf)
        def ld(ref, r0, r1, c0, c1):
            if u32: return pltpu.bitcast(ref[r0//2:r1//2, c0:c1], bf)
            return ref[r0:r1, c0:c1]
        def st(ref, r0, r1, c0, c1, v):
            if u32: ref[r0//2:r1//2, c0:c1] = pltpu.bitcast(v, jnp.uint32)
            else: ref[r0:r1, c0:c1] = v
        dma = not nodma
        w = dma and not nowait

        def step(br, g):
            i = br*8 + g
            s = i % R
            nh = br + 1
            def wait_kv(dst, sem, b):
                if w and b in chunks: c_kv(kB, dst, sem, nh, 0, s, chunks.index(b)).wait()
            def qproj(r0, r1, j):
                st(qb, r0, r1, j*256, (j+1)*256, jnp.dot(xb[br, r0:r1, :], wq[s, :, j*256:(j+1)*256], preferred_element_type=f32).astype(bf))
            def oproj(t):
                if t == 0 and w: c_wo(woA, 0, s).wait()
                acc[pl.ds(pl.multiple_of(br*448, 448), 448), t*128:(t+1)*128] += lax.dot_general(wo[s, :, 0:512], ld(obuf, t*128, (t+1)*128, 0, 512), NT, preferred_element_type=f32)
            if dma: issue(i + D)
            if w: c_wq(wqA, 0, s, 0).wait()
            if xsplit:
                qproj(0, 448, 0)
                if dma:
                    @pl.when(i == 0)
                    def _(): c_x(0, 1).wait()
                qproj(448, 896, 0)
            else: qproj(0, 896, 0)
            if w: c_wq(wqA, 0, s, 1).wait()
            qproj(0, 896, 1)
            items = [(b, j) for b in range(8) for j in range(2)]
            n = len(items)
            ss = {}
            done = 0
            for t in range(n + la):
                if t < n:
                    b, j = items[t]
                    if j == 0: wait_kv(kr, sk, b)
                    ss[t] = scores(ld(qb, b*112, (b+1)*112, j*256, (j+1)*256), kr[s, b, j*br, :, 0:256])
                u = t - la
                if u >= 0:
                    b, j = items[u]
                    if j == 0 and b >= od: oproj(done); done += 1
                    if j == 0: wait_kv(vr, sv, b)
                    if late_a and u == 2*chunks[-2]:
                        @pl.when(i == 15)
                        def _(): c_out(0, 896, 0, 384, 0).start()
                    st(obuf, b*112, (b+1)*112, j*256, (j+1)*256, pv(ss.pop(u), vr[s, b, j*br, :, 0:256]))
            for t in range(done, 7): oproj(t)

        if dma:
            for i in range(D): issue_br(0, i, i, i == 0)
        acc[...] = jnp.zeros_like(acc)
        if dma:
            c_x(0, 0).wait()
            if not xsplit: c_x(0, 1).wait()
        @pl.loop(0, 2)
        def _(br):
            @pl.loop(0, 8)
            def _(g): step(br, g)
            @pl.when(br == 0)
            def _():
                outb[:, 0:384] = acc[0:384, :].T.astype(bf)
                if not late_a: c_out(0, 896, 0, 384, 0).start()
                if dma: c_x(1, 0).wait(); c_x(1, 1).wait()
        if nowait:
            @pl.loop(0, 16)
            def _(i):
                s = i % R
                c_wq(wqA, 0, s, 0).wait(); c_wq(wqA, 0, s, 1).wait(); c_wo(woA, 0, s).wait()
                for c in range(nc):
                    c_kv(kB, kr, sk, i//8+1, 0, s, c).wait(); c_kv(kB, vr, sv, i//8+1, 0, s, c).wait()
        cs = []
        for k in range(len(rows)-1):
            r0, r1 = rows[k], rows[k+1]
            outb[r0:r1, 384:896] = acc[384:896, r0:r1].T.astype(bf)
            cs.append(c_out(r0, r1, 384, 896, k+1)); cs[-1].start()
        c_out(0, 896, 0, 384, 0).wait()
        for c in cs: c.wait()
    def fn(A_x, A_k, A_v, A_wq, A_wo, B_x, B_k, B_v, B_wq, B_wo):
        DMA = pltpu.SemaphoreType.DMA
        qs = pltpu.VMEM((448,512), jnp.uint32) if u32 else pltpu.VMEM((896,512),bf)
        o = pl.pallas_call(kernel, out_shape=jax.ShapeDtypeStruct((896,896), bf),
            in_specs=[pl.BlockSpec(memory_space=pl.ANY)]*10, out_specs=pl.BlockSpec(memory_space=pl.ANY),
            scratch_shapes=[pltpu.VMEM((R,8,2,512,pad),bf), pltpu.VMEM((R,8,2,512,pad),bf),
                pltpu.VMEM((2,896,448),bf), pltpu.VMEM((R,448,512),bf), pltpu.VMEM((R,448,512+wpad),bf),
                qs, qs, pltpu.VMEM((896,896),f32), pltpu.VMEM((896,896),bf),
                DMA((R,nc)), DMA((R,nc)), DMA((R,2)), DMA((R,)), DMA((2,2)), DMA((len(rows),))],
            compiler_params=pltpu.CompilerParams(vmem_limit_bytes=110*2**20, disable_bounds_checks=True, **({"flags": flags} if flags else {})),
            interpret=interpret,
        )(A_x.reshape(896,448), A_k, A_v, A_wq, A_wo.T, B_x.reshape(896,448), B_k, B_v, B_wq, B_wo.T)
        return o.reshape(8,112,896)
    return fn


@jax.jit
def pallas_concat_heads__gqa_block_cached__mha_block_cached__near_ridge_kernel(
        A_x, A_k_cache, A_v_cache, A_wq, A_wo, B_x, B_k_cache, B_v_cache, B_wq, B_wo):
    return build(chunks=(0,3,5,7,8))(A_x, A_k_cache, A_v_cache, A_wq, A_wo, B_x, B_k_cache, B_v_cache, B_wq, B_wo)
```

```python
import jax
import jax.numpy as jnp
import numpy as np
from jax import lax
from jax.experimental import pallas as pl
from jax.experimental.pallas import tpu as pltpu

_B, _SQ, _D, _DH, _SK = 8, 112, 448, 256, 512
_ROWS = _B * _SQ
_PAIR = 2 * _DH
_STEPS = 16
_SLOTS = 8
_AHEAD = 3
_LEAD = 64
_TILES = _ROWS // 128
_TILES_IN_STEP = 3
_A_COLS = 384
_CHUNKS_FIRST = (0, 1, 2, 3, 5, 8)
_CHUNKS_A = (0, 4, 8)
_CHUNKS_B = (0, 4, 6, 7, 8)
_Q_ROWS = (0, 224, 448, 672, 896)
_EPILOGUE = ((0, 3, 3, 5), (3, 5, 5, 6), (5, 7, 6, 7))

_NT = (((1,), (1,)), ((), ()))
_EXP2_SCALE = float(np.log2(np.e) * _DH ** -0.5)


def _softmax_pv(s, v):
    m = jnp.max(s, axis=-1, keepdims=True)
    p = jnp.exp2((s - m) * _EXP2_SCALE)
    l = jnp.sum(p, axis=-1, keepdims=True)
    r = pl.reciprocal(l, approx=True)
    r = r * (2.0 - l * r)
    o = jnp.dot(p.astype(jnp.bfloat16), v, preferred_element_type=jnp.float32)
    return (o * r).astype(jnp.bfloat16)


def _kernel(x_a, k_a, v_a, wq_a, wo_a, x_b, k_b, v_b, wq_b, wo_b, out,
            kv_buf, x_buf, wq_buf, wo_buf, q_buf, o_buf, acc, out_buf, last_step,
            k_sem, v_sem, k_lead_sem, v_lead_sem, wq_sem, wo_sem, x_sem, out_sem):
    copy = pltpu.make_async_copy
    keys = (k_a, k_b, kv_buf.at[0], k_sem, k_lead_sem)
    values = (v_a, v_b, kv_buf.at[1], v_sem, v_lead_sem)

    def aligned(start, size):
        if not isinstance(start, int):
            start = pl.multiple_of(start, size)
        return pl.ds(start, size)

    def per_block(i, fn):
        pl.when(i < 8)(lambda: fn(0))
        pl.when(jnp.logical_and(i >= 8, i < _STEPS))(lambda: fn(1))

    def x_copy(blk, half):
        rows = aligned(half * (_ROWS // 2), _ROWS // 2)
        return copy((x_a, x_b)[blk].at[rows], x_buf.at[blk, rows], x_sem.at[blk, half])

    def wq_copy(i, head):
        cols = aligned(head * _DH, _DH)
        return copy(wq_a.at[:, cols], wq_buf.at[i % _SLOTS, :, cols], wq_sem.at[i % _SLOTS, head])

    def bulk_copy(kv, blk, i, chunks, c):
        src, ring, sem = kv[blk], kv[2], kv[3]
        b0, b1, n = chunks[c], chunks[c + 1], src.shape[2]
        return copy(src.at[b0:b1, i % 8, _LEAD:n], ring.at[i % _SLOTS, b0:b1, _LEAD:n],
                    sem.at[i % _SLOTS, c])

    def lead_copy(kv, i):
        return copy(kv[0].at[:, i % 8, 0:_LEAD], kv[2].at[i % _SLOTS, :, 0:_LEAD],
                    kv[4].at[i % _SLOTS])

    def start_bulk(blk, i, chunks, priority):
        for c in range(len(chunks) - 1):
            bulk_copy(keys, blk, i, chunks, c).start(priority=priority)
            bulk_copy(values, blk, i, chunks, c).start(priority=priority)

    def out_copy(t0, t1, c0, c1, k):
        r0, r1 = t0 * 128, t1 * 128
        return copy(out_buf.at[r0:r1, c0:c1], out.at[r0:r1, c0:c1], out_sem.at[k])

    a_out_copy = lambda: out_copy(0, _TILES, 0, _A_COLS, 0)

    def out_proj(blk, slot, t, first=None):
        rows, cols = aligned(blk * _D, _D), aligned(t * 128, 128)
        prev = acc[rows, cols]
        if first is not None:
            prev = jnp.where(first, 0.0, prev)
        acc[rows, cols] = prev + lax.dot_general(
            wo_buf[slot], o_buf[cols, :], _NT, preferred_element_type=jnp.float32)

    def step(i):
        blk, slot, nxt = i // 8, i % _SLOTS, i + 1
        last_step[0] = i

        def feed_weights(srcs, ring, sem_of, point, points):
            for z in range(16):
                if z * points // 16 == point:
                    rows, c0 = pl.ds((z % 4) * (_D // 4), _D // 4), (z // 4) * 128
                    per_block(nxt, lambda s: copy(
                        srcs[s].at[rows, aligned((nxt % 8) * _PAIR + c0, 128)],
                        ring.at[nxt % _SLOTS, rows, c0:c0 + 128], sem_of(c0)).start())

        def feed_wq(point, points):
            feed_weights((wq_a, wq_b), wq_buf, lambda c0: wq_sem.at[nxt % _SLOTS, c0 // _DH],
                         point, points)

        def feed_wo(point):
            feed_weights((wo_a, wo_b), wo_buf, lambda c0: wo_sem.at[nxt % _SLOTS], point, _TILES)

        def feed_lead(kv, b, half):
            cols = aligned(half * 128, 128)
            per_block(nxt, lambda s: copy(
                kv[s].at[b, nxt % 8, 0:_LEAD, cols], kv[2].at[nxt % _SLOTS, b, 0:_LEAD, cols],
                kv[4].at[nxt % _SLOTS]).start())

        def wait_kv(kv, b):
            if b == 0:
                lead_copy(kv, i).wait()
            for cond, s, chunks in ((i == 0, 0, _CHUNKS_FIRST),
                                    (jnp.logical_and(i > 0, i < 8), 0, _CHUNKS_A),
                                    (i >= 8, 1, _CHUNKS_B)):
                if b in chunks:
                    pl.when(cond)(lambda: bulk_copy(kv, s, i, chunks, chunks.index(b)).wait())

        def load_kv(kv, b, head):
            return kv[2][slot, b, aligned(head * blk * _SK, _SK)]

        ahead = i + _AHEAD

        @pl.when(ahead == 8)
        def _():
            x_copy(1, 0).start(priority=1)
            x_copy(1, 1).start(priority=1)

        per_block(ahead, lambda s: start_bulk(s, ahead, (_CHUNKS_A, _CHUNKS_B)[s], 1))

        for t in range(_TILES_IN_STEP, _TILES):
            out_proj(jnp.maximum(i - 1, 0) // 8, (i + _SLOTS - 1) % _SLOTS, t,
                     jnp.logical_or(i <= 1, i == 9))
            feed_wo(t - _TILES_IN_STEP)

        tile = aligned(jnp.clip(i - 9, 0, _TILES - 1) * 128, 128)
        out_buf[tile, 0:_A_COLS] = acc[0:_A_COLS, tile].T.astype(jnp.bfloat16)

        parts = len(_Q_ROWS) - 1
        for head in range(2):
            cols = aligned(head * _DH, _DH)
            wq_copy(i, head).wait()
            for part in range(parts):
                r0, r1 = _Q_ROWS[part], _Q_ROWS[part + 1]
                if head == 0 and r0 % (_ROWS // 2) == 0:
                    pl.when(i == 0)(lambda: x_copy(0, r0 // (_ROWS // 2)).wait())
                    pl.when(i == 8)(lambda: x_copy(1, r0 // (_ROWS // 2)).wait())
                q = jnp.dot(x_buf[blk, r0:r1, :], wq_buf[slot, :, cols],
                            preferred_element_type=jnp.float32)
                q_buf[r0:r1, cols] = q.astype(jnp.bfloat16)
                feed_wq(head * parts + part, 2 * parts)

        def scores(b, head):
            if head == 0:
                wait_kv(keys, b)
            q = q_buf[aligned(b * _SQ, _SQ), aligned(head * _DH, _DH)]
            s = lax.dot_general(q, load_kv(keys, b, head), _NT,
                                preferred_element_type=jnp.float32)
            feed_lead(keys, b, head)
            return s

        s = scores(0, 0)
        for n in range(2 * _B):
            b, head = divmod(n, 2)
            s_next = scores(*divmod(n + 1, 2)) if n + 1 < 2 * _B else None
            if head == 0:
                t = b - 2
                if 0 <= t < _TILES_IN_STEP:
                    if t == 0:
                        copy(wo_a.at[:, 0:_PAIR], wo_buf.at[slot], wo_sem.at[slot]).wait()
                    out_proj(blk, slot, t, i % 8 == 0)
                    feed_wo(_TILES - _TILES_IN_STEP + t)
                wait_kv(values, b)
                if b == _B - 1:
                    pl.when(i == _STEPS - 1)(lambda: a_out_copy().start())
            o_buf[aligned(b * _SQ, _SQ), aligned(head * _DH, _DH)] = _softmax_pv(
                s, load_kv(values, b, head))
            feed_lead(values, b, head)
            s = s_next

    wq_copy(0, 0).start()
    pl.loop(0, 2)(lambda half: x_copy(0, half).start())
    wq_copy(0, 1).start()
    lead_copy(keys, 0).start()
    lead_copy(values, 0).start()

    @pl.loop(0, 2)
    def _(half):
        rows = aligned(half * (_D // 2), _D // 2)
        copy(wo_a.at[rows, 0:_PAIR], wo_buf.at[0, rows], wo_sem.at[0]).start()

    start_bulk(0, 0, _CHUNKS_FIRST, 0)
    for i in range(1, _AHEAD):
        start_bulk(0, i, _CHUNKS_A, 1)

    pl.loop(0, _STEPS)(step)

    out_copies = [out_copy(t0, t1, _A_COLS, 2 * _D, k + 1)
                  for k, (t0, t1, _, _) in enumerate(_EPILOGUE)]

    def finish(k):
        t0, t1, p0, p1 = _EPILOGUE[k]

        def write_back():
            rows = slice(t0 * 128, t1 * 128)
            out_buf[rows, _A_COLS:2 * _D] = acc[_A_COLS:2 * _D, rows].T.astype(jnp.bfloat16)
            out_copies[k].start()

        if t1 <= p0:
            write_back()
        for t in range(p0, p1):
            out_proj(1, (_STEPS - 1) % _SLOTS, t)
        if t1 > p0:
            write_back()

    pl.when(last_step[0] == _STEPS - 1)(lambda: finish(0))
    for k in range(1, len(_EPILOGUE)):
        finish(k)
    a_out_copy().wait()
    for c in out_copies:
        c.wait()


def _attention_blocks(a_x, a_k, a_v, a_wq, a_wo, b_x, b_k, b_v, b_wq, b_wo, interpret=False):
    bf16 = jnp.bfloat16
    dma = pltpu.SemaphoreType.DMA
    chunks = max(len(_CHUNKS_FIRST), len(_CHUNKS_A), len(_CHUNKS_B)) - 1
    out = pl.pallas_call(
        _kernel,
        out_shape=jax.ShapeDtypeStruct((_ROWS, 2 * _D), bf16),
        in_specs=[pl.BlockSpec(memory_space=pl.ANY)] * 10,
        out_specs=pl.BlockSpec(memory_space=pl.ANY),
        scratch_shapes=[
            pltpu.VMEM((2, _SLOTS, _B, 2 * _SK, _DH), bf16),
            pltpu.VMEM((2, _ROWS, _D), bf16),
            pltpu.VMEM((_SLOTS, _D, _PAIR), bf16),
            pltpu.VMEM((_SLOTS, _D, _PAIR), bf16),
            pltpu.VMEM((_ROWS, _PAIR), bf16),
            pltpu.VMEM((_ROWS, _PAIR), bf16),
            pltpu.VMEM((2 * _D, _ROWS), jnp.float32),
            pltpu.VMEM((_ROWS, 2 * _D), bf16),
            pltpu.SMEM((1,), jnp.int32),
            dma((_SLOTS, chunks)), dma((_SLOTS, chunks)), dma((_SLOTS,)), dma((_SLOTS,)),
            dma((_SLOTS, 2)), dma((_SLOTS,)), dma((2, 2)), dma((len(_EPILOGUE) + 1,)),
        ],
        compiler_params=pltpu.CompilerParams(
            vmem_limit_bytes=110 * 2**20,
            disable_bounds_checks=True,
            disable_semaphore_checks=True,
            flags={"XLA_TPU_RESCHEDULE_DMA_DONES": True},
        ),
        interpret=interpret,
    )(
        a_x.reshape(_ROWS, _D), a_k, a_v, a_wq, a_wo.T,
        b_x.reshape(_ROWS, _D),
        b_k.reshape(_B, 8, 2 * _SK, _DH), b_v.reshape(_B, 8, 2 * _SK, _DH), b_wq, b_wo.T,
    )
    return out.reshape(_B, _SQ, 2 * _D)


@jax.jit
def pallas_concat_heads__gqa_block_cached__mha_block_cached__near_ridge_kernel(
    A_x: jax.Array,
    A_k_cache: jax.Array,
    A_v_cache: jax.Array,
    A_wq: jax.Array,
    A_wo: jax.Array,
    B_x: jax.Array,
    B_k_cache: jax.Array,
    B_v_cache: jax.Array,
    B_wq: jax.Array,
    B_wo: jax.Array,
):
    return _attention_blocks(A_x, A_k_cache, A_v_cache, A_wq, A_wo,
                             B_x, B_k_cache, B_v_cache, B_wq, B_wo)
```

```python
import jax
import jax.numpy as jnp
import numpy as np
from jax import lax
from jax.experimental import pallas as pl
from jax.experimental.pallas import tpu as pltpu

_B, _SQ, _D, _DH, _SK = 8, 112, 448, 256, 512
_ROWS = _B * _SQ
_PAIR = 2 * _DH
_STEPS = 16
_SLOTS = 8
_AHEAD = 3
_LEAD = 64
_TILES = _ROWS // 128
_TILES_IN_STEP = 3
_A_COLS = 384
_CHUNKS_FIRST = (0, 1, 2, 3, 5, 7, 8)
_CHUNKS_A = (0, 4, 8)
_CHUNKS_B = (0, 4, 6, 7, 8)
_Q_ROWS = tuple(range(0, _ROWS + 1, _SQ))
_EPILOGUE = ((0, 3, 3, 5), (3, 5, 5, 6), (5, 7, 6, 7))

_NT = (((1,), (1,)), ((), ()))
_EXP2_SCALE = float(np.log2(np.e) * _DH ** -0.5)


def _softmax_pv(s, v):
    m = jnp.max(s, axis=-1, keepdims=True)
    p = jnp.exp2((s - m) * _EXP2_SCALE)
    l = jnp.sum(p, axis=-1, keepdims=True)
    r = pl.reciprocal(l, approx=True)
    r = r * (2.0 - l * r)
    o = jnp.dot(p.astype(jnp.bfloat16), v, preferred_element_type=jnp.float32)
    return (o * r).astype(jnp.bfloat16)


def _kernel(x_a, k_a, v_a, wq_a, wo_a, x_b, k_b, v_b, wq_b, wo_b, out,
            kv_buf, x_buf, wq_buf, wo_buf, q_buf, o_buf, acc, out_buf, last_step,
            k_sem, v_sem, k_lead_sem, v_lead_sem, wq_sem, wo_sem, x_sem, out_sem):
    copy = pltpu.make_async_copy
    keys = (k_a, k_b, kv_buf.at[0], k_sem, k_lead_sem)
    values = (v_a, v_b, kv_buf.at[1], v_sem, v_lead_sem)

    def aligned(start, size):
        if not isinstance(start, int):
            start = pl.multiple_of(start, size)
        return pl.ds(start, size)

    def per_block(i, fn):
        pl.when(i < 8)(lambda: fn(0))
        pl.when(jnp.logical_and(i >= 8, i < _STEPS))(lambda: fn(1))

    def x_copy(blk, half):
        rows = aligned(half * (_ROWS // 2), _ROWS // 2)
        return copy((x_a, x_b)[blk].at[rows], x_buf.at[blk, rows], x_sem.at[blk, half])

    def wq_copy(i, head):
        cols = aligned(head * _DH, _DH)
        return copy(wq_a.at[:, cols], wq_buf.at[i % _SLOTS, :, cols], wq_sem.at[i % _SLOTS, head])

    def bulk_copy(kv, blk, i, chunks, c):
        src, ring, sem = kv[blk], kv[2], kv[3]
        b0, b1, n = chunks[c], chunks[c + 1], src.shape[2]
        k0 = 0 if chunks is _CHUNKS_FIRST else _LEAD
        return copy(src.at[b0:b1, i % 8, k0:n], ring.at[i % _SLOTS, b0:b1, k0:n],
                    sem.at[i % _SLOTS, c])

    def lead_copy(kv, i):
        return copy(kv[0].at[:, i % 8, 0:_LEAD], kv[2].at[i % _SLOTS, :, 0:_LEAD],
                    kv[4].at[i % _SLOTS])

    def start_bulk(i, chunks, priority):
        for c in range(len(chunks) - 1):
            bulk_copy(keys, 0, i, chunks, c).start(priority=priority)
            bulk_copy(values, 0, i, chunks, c).start(priority=priority)

    def out_copy(t0, t1, c0, c1, k):
        r0, r1 = t0 * 128, t1 * 128
        return copy(out_buf.at[r0:r1, c0:c1], out.at[r0:r1, c0:c1], out_sem.at[k])

    a_out_copy = lambda: out_copy(0, _TILES, 0, _A_COLS, 0)

    def out_proj(blk, slot, t, first=None, feed=None):
        cols, n = aligned(t * 128, 128), _D // 2
        for half in range(2):
            rows = aligned(blk * _D + half * n, n)
            prev = acc[rows, cols]
            if first is not None:
                prev = jnp.where(first, 0.0, prev)
            acc[rows, cols] = prev + lax.dot_general(
                wo_buf[slot, half * n:(half + 1) * n], o_buf[cols, :], _NT,
                preferred_element_type=jnp.float32)
            if feed is not None:
                feed(half)

    def step(i):
        blk, slot, nxt = i // 8, i % _SLOTS, i + 1
        last_step[0] = i

        def feed_weights(srcs, ring, sem_of, point, points):
            for z in range(16):
                if z * points // 16 == point:
                    rows, c0 = pl.ds((z % 4) * (_D // 4), _D // 4), (z // 4) * 128
                    per_block(nxt, lambda s: copy(
                        srcs[s].at[rows, aligned((nxt % 8) * _PAIR + c0, 128)],
                        ring.at[nxt % _SLOTS, rows, c0:c0 + 128], sem_of(c0)).start())

        def feed_wq(point, points):
            feed_weights((wq_a, wq_b), wq_buf, lambda c0: wq_sem.at[nxt % _SLOTS, c0 // _DH],
                         point, points)

        def feed_wo(point):
            feed_weights((wo_a, wo_b), wo_buf, lambda c0: wo_sem.at[nxt % _SLOTS], point,
                         2 * _TILES)

        def feed_lead(kv, b, half):
            cols = aligned(half * 128, 128)
            per_block(nxt, lambda s: copy(
                kv[s].at[b, nxt % 8, 0:_LEAD, cols], kv[2].at[nxt % _SLOTS, b, 0:_LEAD, cols],
                kv[4].at[nxt % _SLOTS]).start())

        def wait_kv(kv, b):
            if b == 0:
                pl.when(i > 0)(lambda: lead_copy(kv, i).wait())
            for cond, s, chunks in ((i == 0, 0, _CHUNKS_FIRST),
                                    (jnp.logical_and(i > 0, i < 8), 0, _CHUNKS_A),
                                    (i >= 8, 1, _CHUNKS_B)):
                if b in chunks:
                    pl.when(cond)(lambda: bulk_copy(kv, s, i, chunks, chunks.index(b)).wait())

        def load_kv(kv, b, head):
            return kv[2][slot, b, aligned(head * blk * _SK, _SK)]

        ahead = i + _AHEAD

        @pl.when(ahead == 8)
        def _():
            x_copy(1, 0).start(priority=1)
            x_copy(1, 1).start(priority=1)

        def feed_bulk(kv, c):
            def start(s):
                chunks = (_CHUNKS_A, _CHUNKS_B)[s]
                if c < len(chunks) - 1:
                    bulk_copy(kv, s, ahead, chunks, c).start(priority=1)
            per_block(ahead, start)

        for t in range(_TILES_IN_STEP, _TILES):
            out_proj(jnp.maximum(i - 1, 0) // 8, (i + _SLOTS - 1) % _SLOTS, t,
                     jnp.logical_or(i <= 1, i == 9),
                     lambda half: feed_wo(2 * (t - _TILES_IN_STEP) + half))

        tile = aligned(jnp.clip(i - 9, 0, _TILES - 1) * 128, 128)
        out_buf[tile, 0:_A_COLS] = acc[0:_A_COLS, tile].T.astype(jnp.bfloat16)

        parts = len(_Q_ROWS) - 1
        for head in range(2):
            cols = aligned(head * _DH, _DH)
            wq_copy(i, head).wait()
            for part in range(parts):
                r0, r1 = _Q_ROWS[part], _Q_ROWS[part + 1]
                if head == 0 and r0 % (_ROWS // 2) == 0:
                    pl.when(i == 0)(lambda: x_copy(0, r0 // (_ROWS // 2)).wait())
                    pl.when(i == 8)(lambda: x_copy(1, r0 // (_ROWS // 2)).wait())
                q = jnp.dot(x_buf[blk, r0:r1, :], wq_buf[slot, :, cols],
                            preferred_element_type=jnp.float32)
                q_buf[r0:r1, cols] = q.astype(jnp.bfloat16)
                feed_wq(head * parts + part, 2 * parts)

        def scores(b, head):
            if head == 0:
                wait_kv(keys, b)
            q = q_buf[aligned(b * _SQ, _SQ), aligned(head * _DH, _DH)]
            s = lax.dot_general(q, load_kv(keys, b, head), _NT,
                                preferred_element_type=jnp.float32)
            feed_lead(keys, b, head)
            if head == 0:
                feed_bulk(keys, b)
            return s

        s = scores(0, 0)
        for n in range(2 * _B):
            b, head = divmod(n, 2)
            s_next = scores(*divmod(n + 1, 2)) if n + 1 < 2 * _B else None
            if head == 0:
                t = b - 2
                if 0 <= t < _TILES_IN_STEP:
                    if t == 0:
                        copy(wo_a.at[:, 0:_PAIR], wo_buf.at[slot], wo_sem.at[slot]).wait()
                    out_proj(blk, slot, t, i % 8 == 0,
                             lambda half: feed_wo(2 * (_TILES - _TILES_IN_STEP + t) + half))
                wait_kv(values, b)
                if b == _B - 1:
                    pl.when(i == _STEPS - 1)(lambda: a_out_copy().start())
            o_buf[aligned(b * _SQ, _SQ), aligned(head * _DH, _DH)] = _softmax_pv(
                s, load_kv(values, b, head))
            feed_lead(values, b, head)
            if head == 0:
                feed_bulk(values, b)
            s = s_next

    wq_copy(0, 0).start()
    pl.loop(0, 2)(lambda half: x_copy(0, half).start())
    wq_copy(0, 1).start()

    @pl.loop(0, 2)
    def _(half):
        rows = aligned(half * (_D // 2), _D // 2)
        copy(wo_a.at[rows, 0:_PAIR], wo_buf.at[0, rows], wo_sem.at[0]).start()

    start_bulk(0, _CHUNKS_FIRST, 0)
    for i in range(1, _AHEAD):
        start_bulk(i, _CHUNKS_A, 1)

    pl.loop(0, _STEPS)(step)

    out_copies = [out_copy(t0, t1, _A_COLS, 2 * _D, k + 1)
                  for k, (t0, t1, _, _) in enumerate(_EPILOGUE)]

    def finish(k):
        t0, t1, p0, p1 = _EPILOGUE[k]

        def write_back():
            rows = slice(t0 * 128, t1 * 128)
            out_buf[rows, _A_COLS:2 * _D] = acc[_A_COLS:2 * _D, rows].T.astype(jnp.bfloat16)
            out_copies[k].start()

        if t1 <= p0:
            write_back()
        for t in range(p0, p1):
            out_proj(1, (_STEPS - 1) % _SLOTS, t)
        if t1 > p0:
            write_back()

    pl.when(last_step[0] == _STEPS - 1)(lambda: finish(0))
    for k in range(1, len(_EPILOGUE)):
        finish(k)
    a_out_copy().wait()
    for c in out_copies:
        c.wait()


def _attention_blocks(a_x, a_k, a_v, a_wq, a_wo, b_x, b_k, b_v, b_wq, b_wo, interpret=False):
    bf16 = jnp.bfloat16
    dma = pltpu.SemaphoreType.DMA
    chunks = max(len(_CHUNKS_FIRST), len(_CHUNKS_A), len(_CHUNKS_B)) - 1
    out = pl.pallas_call(
        _kernel,
        out_shape=jax.ShapeDtypeStruct((_ROWS, 2 * _D), bf16),
        in_specs=[pl.BlockSpec(memory_space=pl.ANY)] * 10,
        out_specs=pl.BlockSpec(memory_space=pl.ANY),
        scratch_shapes=[
            pltpu.VMEM((2, _SLOTS, _B, 2 * _SK, _DH), bf16),
            pltpu.VMEM((2, _ROWS, _D), bf16),
            pltpu.VMEM((_SLOTS, _D, _PAIR), bf16),
            pltpu.VMEM((_SLOTS, _D, _PAIR), bf16),
            pltpu.VMEM((_ROWS, _PAIR), bf16),
            pltpu.VMEM((_ROWS, _PAIR), bf16),
            pltpu.VMEM((2 * _D, _ROWS), jnp.float32),
            pltpu.VMEM((_ROWS, 2 * _D), bf16),
            pltpu.SMEM((1,), jnp.int32),
            dma((_SLOTS, chunks)), dma((_SLOTS, chunks)), dma((_SLOTS,)), dma((_SLOTS,)),
            dma((_SLOTS, 2)), dma((_SLOTS,)), dma((2, 2)), dma((len(_EPILOGUE) + 1,)),
        ],
        compiler_params=pltpu.CompilerParams(
            vmem_limit_bytes=110 * 2**20,
            disable_bounds_checks=True,
            disable_semaphore_checks=True,
            flags={"XLA_TPU_RESCHEDULE_DMA_DONES": True},
        ),
        interpret=interpret,
    )(
        a_x.reshape(_ROWS, _D), a_k, a_v, a_wq, a_wo.T,
        b_x.reshape(_ROWS, _D),
        b_k.reshape(_B, 8, 2 * _SK, _DH), b_v.reshape(_B, 8, 2 * _SK, _DH), b_wq, b_wo.T,
    )
    return out.reshape(_B, _SQ, 2 * _D)


@jax.jit
def pallas_concat_heads__gqa_block_cached__mha_block_cached__near_ridge_kernel(
    A_x: jax.Array,
    A_k_cache: jax.Array,
    A_v_cache: jax.Array,
    A_wq: jax.Array,
    A_wo: jax.Array,
    B_x: jax.Array,
    B_k_cache: jax.Array,
    B_v_cache: jax.Array,
    B_wq: jax.Array,
    B_wo: jax.Array,
):
    return _attention_blocks(A_x, A_k_cache, A_v_cache, A_wq, A_wo,
                             B_x, B_k_cache, B_v_cache, B_wq, B_wo)
```
